```python
import jax
import jax.numpy as jnp

def _softmax(x, axis=-1):
    return jax.nn.softmax(x, axis=axis)
def _gelu(x):
    return jax.nn.gelu(x, approximate=True)
def _silu(x):
    return jax.nn.silu(x)
def _sigmoid(x):
    return jax.nn.sigmoid(x)
def _layernorm(x, axis=-1, eps=1e-5):
    m = jnp.mean(x, axis=axis, keepdims=True)
    v = jnp.var(x, axis=axis, keepdims=True)
    return (x - m) / jnp.sqrt(v + eps)
def _scatter_add(tgt, idx, src, axis=0):
    return tgt.at[idx].add(src)
def _segment_sum(src, seg, n):
    return jax.ops.segment_sum(src, seg, n)
class _Rng:
    def __init__(self, key):
        self._k = key
    def _next(self):
        self._k, sub = jax.random.split(self._k)
        return sub
    def normal(self, shape):
        return jax.random.normal(self._next(), shape, dtype=jnp.bfloat16)
    def randint(self, lo, hi, shape):
        return jax.random.randint(self._next(), shape, lo, hi, dtype=jnp.int32)
    def uniform(self, shape, lo=0.0, hi=1.0):
        return jax.random.uniform(self._next(), shape, jnp.bfloat16, lo, hi)
    def permutation(self, n):
        return jax.random.permutation(self._next(), n)


kernel_name = 'sequential_preLN__sliding_block_cached__moe_arch_mod__decode'

def setup_inputs():
    _rng = _Rng(jax.random.key(int.from_bytes(__import__("os").urandom(4), "little")))
    _w = (lambda a: (lambda t: t.astype(jnp.bfloat16) if jnp.issubdtype(t.dtype, jnp.floating) else t)(jnp.asarray(a)))
    def _A_setup():
        B, Sq, D = 1, 1, 640
        Hq, Hkv, Sk, Dh = 32, 32, 32768, 192
        assert Hq % Hkv == 0, (Hq, Hkv)
        return {
            "x": _w((lambda *s: _rng.normal(s) * 0.05)(B, Sq, D)),
            "k_cache": _w((lambda *s: _rng.normal(s) * 0.05)(B, Hkv, Sk, Dh)),
            "v_cache": _w((lambda *s: _rng.normal(s) * 0.05)(B, Hkv, Sk, Dh)),
            "wq": _w((lambda *s: _rng.normal(s) * 0.05)(D, Hq * Dh) * (D ** -0.5)),
            "wo": _w((lambda *s: _rng.normal(s) * 0.05)(Hq * Dh, D) * ((Hq * Dh) ** -0.5)),
        }
    _A_in = _A_setup()

    def _B_setup():
        B, S, D, F, C = 1, 1, 640, 1536, 1
        return {
            "x": _w((lambda *s: _rng.normal(s) * 0.05)(B, S, D)),
            "w_r": _w((lambda *s: _rng.normal(s) * 0.05)(D)),
            "w_gate": _w((lambda *s: _rng.normal(s) * 0.05)(D, F)),
            "w_up": _w((lambda *s: _rng.normal(s) * 0.05)(D, F)),
            "w_down": _w((lambda *s: _rng.normal(s) * 0.05)(F, D)),
        }
    _B_in = _B_setup()

    return {
        "A_x": _A_in["x"],
        "A_k_cache": _A_in["k_cache"],
        "A_v_cache": _A_in["v_cache"],
        "A_wq": _A_in["wq"],
        "A_wo": _A_in["wo"],
        "B_x": _B_in["x"],
        "B_w_r": _B_in["w_r"],
        "B_w_gate": _B_in["w_gate"],
        "B_w_up": _B_in["w_up"],
        "B_w_down": _B_in["w_down"],
    }

def reference(A_x, A_k_cache, A_v_cache, A_wq, A_wo, B_x, B_w_r, B_w_gate, B_w_up, B_w_down):
    def _A_ref(x, k_cache, v_cache, wq, wo):
        B, Sq, D = x.shape
        Hq, Dh = 32, 192
        Hkv, Sk = k_cache.shape[1], k_cache.shape[2]
        W = min(4096, max(256, Sk // 4))
        rep = Hq // Hkv
        q = (lambda x, *d: x.transpose(*d))((x @ wq).reshape(B, Sq, Hq, Dh), 0, 2, 1, 3)
        k = jnp.repeat(k_cache[:, :, Sk - W:, :], rep, axis=1)
        v = jnp.repeat(v_cache[:, :, Sk - W:, :], rep, axis=1)
        scores = jnp.einsum("bhqd,bhkd->bhqk", q, k) * (Dh ** -0.5)
        p = _softmax(scores, axis=-1)
        o = jnp.einsum("bhqk,bhkd->bhqd", p, v)
        return (lambda x, *d: x.transpose(*d))(o, 0, 2, 1, 3).reshape(B, Sq, Hq * Dh) @ wo

    def _B_ref(x, w_r, w_gate, w_up, w_down):
        B, S, D = x.shape
        C = 1
        r = x @ w_r
        idx = jnp.argsort(-r, axis=-1)[:, :C]
        idx_e = jnp.repeat(idx.reshape(B, C, 1), D, axis=2)
        x_sel = jnp.take_along_axis(x, idx_e, axis=1)
        g = _silu(x_sel @ w_gate)
        u = x_sel @ w_up
        y = (g * u) @ w_down
        r_sel = _sigmoid(jnp.take_along_axis(r, idx, axis=1))
        y = y * r_sel.reshape(B, C, 1)
        b_off = (jnp.arange(B) * S).reshape(B, 1)
        flat_idx = (idx + b_off).reshape(B * C)
        zero = (x * 0.0).reshape(B * S, D)
        upd = _scatter_add(zero, flat_idx, y.reshape(B * C, D), axis=0)
        return x + upd.reshape(B, S, D)

    x = A_x
    h = x + _A_ref(_layernorm(x, axis=-1), A_k_cache, A_v_cache, A_wq, A_wo)
    h2 = h + _B_ref(_layernorm(h, axis=-1), B_w_r, B_w_gate, B_w_up, B_w_down)
    return h2
```

```python
import jax
import jax.numpy as jnp
from jax import lax
import jax.experimental.pallas as pl
import jax.experimental.pallas.tpu as pltpu

NBUF = 4
DH = 192
G = 2 * DH
BF, F32 = jnp.bfloat16, jnp.float32


def _ln(x):
    m = jnp.mean(x, axis=-1, keepdims=True)
    d = x - m
    v = jnp.mean(d * d, axis=-1, keepdims=True)
    return d / jnp.sqrt(v + 1e-5)


def _mm(a, b):
    return jnp.dot(a.astype(BF), b, preferred_element_type=F32)


def _body(x_ref, wr_ref, kt, vt, wq_h, wo_h, wg_h, wu_h, wd_h, o_ref,
          kb, vb, wq, wo, wg, wu, wd, qs, ks, vs, ws):
    R, S = kt.shape
    W = kb.shape[-1]
    D = x_ref.shape[-1]
    NP = R // G

    def cp(src, dst, sem, i):
        s = i % NBUF
        r = i * G if isinstance(i, int) else pl.multiple_of(i * G, G)
        return pltpu.make_async_copy(
            src.at[pl.ds(r, G), pl.ds(S - W, W)], dst.at[s], sem.at[s])

    wc = [pltpu.make_async_copy(a, b, ws.at[n]) for n, (a, b) in enumerate(
        [(wq_h, wq), (wo_h, wo), (wg_h, wg), (wu_h, wu), (wd_h, wd)])]
    cp(kt, kb, ks, 0).start()
    wc[0].start()
    cp(vt, vb, vs, 0).start()
    wc[1].start()
    for i in range(1, NBUF):
        cp(kt, kb, ks, i).start()
        cp(vt, vb, vs, i).start()

    x = jnp.broadcast_to(x_ref[...].astype(F32), (8, D))
    xn = _ln(x)
    diag = (lax.broadcasted_iota(jnp.int32, (8, G), 1) // DH
            == lax.broadcasted_iota(jnp.int32, (8, G), 0))
    wc[0].wait()
    for i in range(NP):
        q = _mm(xn, wq[:, i * G:(i + 1) * G])
        qs[i] = jnp.where(diag, q, 0.0)
    wc[1].wait()

    def step(i, acc):
        s = i % NBUF
        cp(kt, kb, ks, i).wait()
        sc = _mm(qs[i], kb[s]) * (DH ** -0.5)

        @pl.when(i + NBUF < NP)
        def _():
            cp(kt, kb, ks, i + NBUF).start()

        e = jnp.exp(sc - jnp.max(sc, axis=-1, keepdims=True))
        p = e * (1.0 / jnp.sum(e, axis=-1, keepdims=True))
        cp(vt, vb, vs, i).wait()
        o = lax.dot_general(p.astype(BF), vb[s], (((1,), (1,)), ((), ())),
                            preferred_element_type=F32)

        @pl.when(i + NBUF < NP)
        def _():
            cp(vt, vb, vs, i + NBUF).start()

        @pl.when(i + NBUF == NP)
        def _():
            for c in wc[2:]:
                c.start()

        o = jnp.where(diag, o, 0.0)
        return acc + _mm(o, wo[pl.ds(pl.multiple_of(i * G, G), G), :])

    acc = lax.fori_loop(0, NP, step, jnp.zeros((8, D), F32))
    h = x + jnp.sum(acc, axis=0, keepdims=True)
    hn = _ln(h)
    r = jnp.sum(hn * wr_ref[...].astype(F32), axis=-1, keepdims=True)
    wc[2].wait()
    g = _mm(hn, wg[...])
    g = g * jax.nn.sigmoid(g)
    wc[3].wait()
    u = _mm(hn, wu[...])
    wc[4].wait()
    y = _mm(g * u, wd[...]) * jax.nn.sigmoid(r)
    o_ref[...] = (h + hn + y)[0:1].astype(o_ref.dtype)


@jax.jit
def pallas_sequential_preLN__sliding_block_cached__moe_arch_mod__decode_kernel(
    A_x, A_k_cache, A_v_cache, A_wq, A_wo, B_x, B_w_r, B_w_gate, B_w_up, B_w_down,
):
    _, H, S, dh = A_k_cache.shape
    D = A_x.shape[-1]
    W = min(4096, max(256, S // 4))
    kt = jnp.swapaxes(A_k_cache, 2, 3).reshape(H * dh, S)
    vt = jnp.swapaxes(A_v_cache, 2, 3).reshape(H * dh, S)
    hbm = pl.BlockSpec(memory_space=pl.ANY)
    vm = pl.BlockSpec(memory_space=pltpu.VMEM)
    big = (A_wq, A_wo, B_w_gate, B_w_up, B_w_down)
    out = pl.pallas_call(
        _body,
        in_specs=[vm, vm] + [hbm] * 7,
        out_specs=vm,
        out_shape=jax.ShapeDtypeStruct((1, D), A_x.dtype),
        scratch_shapes=[pltpu.VMEM((NBUF, G, W), BF)] * 2
        + [pltpu.VMEM(w.shape, BF) for w in big]
        + [pltpu.VMEM((H * dh // G, 8, G), F32)]
        + [pltpu.SemaphoreType.DMA((NBUF,))] * 2
        + [pltpu.SemaphoreType.DMA((5,))],
        compiler_params=pltpu.CompilerParams(vmem_limit_bytes=100 * 2**20),
    )(A_x.reshape(1, D), B_w_r.reshape(1, D), kt, vt, *big)
    return out.reshape(A_x.shape)
```

```python
import jax
import jax.numpy as jnp
from jax import lax
import jax.experimental.pallas as pl
import jax.experimental.pallas.tpu as pltpu

NBUF = 3
SG = 1
DH = 192
G = 2 * DH
BF, F32 = jnp.bfloat16, jnp.float32


def _ln(x):
    m = jnp.mean(x, axis=-1, keepdims=True)
    d = x - m
    v = jnp.mean(d * d, axis=-1, keepdims=True)
    return d / jnp.sqrt(v + 1e-5)


def _mm(a, b):
    return jnp.dot(a.astype(BF), b, preferred_element_type=F32)


def _body(x_ref, wr_ref, kt, vt, wq_h, wo_h, wg_h, wu_h, wd_h, o_ref,
          kb, vb, wq, wo, wg, wu, wd, qs, ks, vs, ws):
    R, S = kt.shape
    W = kb.shape[-1]
    D = x_ref.shape[-1]
    NP = R // G

    def cp(src, dst, sem, i):
        s = i % NBUF
        r = i * G if isinstance(i, int) else pl.multiple_of(i * G, G)
        return pltpu.make_async_copy(
            src.at[pl.ds(r, G), pl.ds(S - W, W)], dst.at[s], sem.at[s])

    wc = [pltpu.make_async_copy(a, b, ws.at[n]) for n, (a, b) in enumerate(
        [(wq_h, wq), (wo_h, wo), (wg_h, wg), (wu_h, wu), (wd_h, wd)])]
    cp(kt, kb, ks, 0).start()
    wc[0].start()
    cp(vt, vb, vs, 0).start()
    wc[1].start()
    for i in range(1, NBUF):
        cp(kt, kb, ks, i).start()
        cp(vt, vb, vs, i).start()

    x = jnp.broadcast_to(x_ref[...].astype(F32), (8, D))
    xn = _ln(x)
    diag = (lax.broadcasted_iota(jnp.int32, (8, G), 1) // DH
            == lax.broadcasted_iota(jnp.int32, (8, G), 0))
    wc[0].wait()
    for i in range(NP):
        q = _mm(xn, wq[:, i * G:(i + 1) * G])
        qs[i] = jnp.where(diag, q, 0.0)
    wc[1].wait()

    def step(i, acc):
        s = i % NBUF
        cp(kt, kb, ks, i).wait()
        sc = _mm(qs[i], kb[s]) * (DH ** -0.5)

        @pl.when(i + NBUF < NP)
        def _():
            cp(kt, kb, ks, i + NBUF).start()

        e = jnp.exp(sc - jnp.max(sc, axis=-1, keepdims=True))
        p = e * (1.0 / jnp.sum(e, axis=-1, keepdims=True))
        cp(vt, vb, vs, i).wait()
        o = lax.dot_general(p.astype(BF), vb[s], (((1,), (1,)), ((), ())),
                            preferred_element_type=F32)

        @pl.when(i + NBUF < NP)
        def _():
            cp(vt, vb, vs, i + NBUF).start()

        for n in range(3):
            pl.when(i + NBUF == NP - (2, 1, 0)[n] * SG)(wc[2 + n].start)

        o = jnp.where(diag, o, 0.0)
        return acc + _mm(o, wo[pl.ds(pl.multiple_of(i * G, G), G), :])

    acc = lax.fori_loop(0, NP, step, jnp.zeros((8, D), F32))
    h = x + jnp.sum(acc, axis=0, keepdims=True)
    hn = _ln(h)
    r = jnp.sum(hn * wr_ref[...].astype(F32).reshape(1, D), axis=-1, keepdims=True)
    wc[2].wait()
    g = _mm(hn, wg[...])
    g = g * jax.nn.sigmoid(g)
    wc[3].wait()
    u = _mm(hn, wu[...])
    wc[4].wait()
    y = _mm(g * u, wd[...]) * jax.nn.sigmoid(r)
    o_ref[...] = (h + hn + y)[0:1].astype(o_ref.dtype)


@jax.jit
def pallas_sequential_preLN__sliding_block_cached__moe_arch_mod__decode_kernel(
    A_x, A_k_cache, A_v_cache, A_wq, A_wo, B_x, B_w_r, B_w_gate, B_w_up, B_w_down,
):
    _, H, S, dh = A_k_cache.shape
    D = A_x.shape[-1]
    W = min(4096, max(256, S // 4))
    kt = jnp.swapaxes(A_k_cache, 2, 3).reshape(H * dh, S)
    vt = jnp.swapaxes(A_v_cache, 2, 3).reshape(H * dh, S)
    hbm = pl.BlockSpec(memory_space=pl.ANY)
    vm = pl.BlockSpec(memory_space=pltpu.VMEM)
    big = (A_wq, A_wo, B_w_gate, B_w_up, B_w_down)
    out = pl.pallas_call(
        _body,
        in_specs=[vm, vm] + [hbm] * 7,
        out_specs=vm,
        out_shape=jax.ShapeDtypeStruct((1, D), A_x.dtype),
        scratch_shapes=[pltpu.VMEM((NBUF, G, W), BF)] * 2
        + [pltpu.VMEM(w.shape, BF) for w in big]
        + [pltpu.VMEM((H * dh // G, 8, G), F32)]
        + [pltpu.SemaphoreType.DMA((NBUF,))] * 2
        + [pltpu.SemaphoreType.DMA((5,))],
        compiler_params=pltpu.CompilerParams(vmem_limit_bytes=100 * 2**20),
    )(A_x.reshape(1, D), B_w_r, kt, vt, *big)
    return out.reshape(A_x.shape)
```
